```python
import os as _os
_os.environ.setdefault("JAX_PLATFORMS", "cpu")
import jax
import jax.numpy as jnp

def _softmax(x, axis=-1):
    return jax.nn.softmax(x, axis=axis)
def _gelu(x):
    return jax.nn.gelu(x, approximate=True)
def _silu(x):
    return jax.nn.silu(x)
def _sigmoid(x):
    return jax.nn.sigmoid(x)
def _layernorm(x, axis=-1, eps=1e-5):
    m = jnp.mean(x, axis=axis, keepdims=True)
    v = jnp.var(x, axis=axis, keepdims=True)
    return (x - m) / jnp.sqrt(v + eps)
def _scatter_add(tgt, idx, src, axis=0):
    return tgt.at[idx].add(src)
def _segment_sum(src, seg, n):
    return jax.ops.segment_sum(src, seg, n)
class _Rng:
    def __init__(self, key):
        self._k = key
    def _next(self):
        self._k, sub = jax.random.split(self._k)
        return sub
    def normal(self, shape):
        return jax.random.normal(self._next(), shape, dtype=jnp.bfloat16)
    def randint(self, lo, hi, shape):
        return jax.random.randint(self._next(), shape, lo, hi, dtype=jnp.int32)
    def uniform(self, shape, lo=0.0, hi=1.0):
        return jax.random.uniform(self._next(), shape, jnp.bfloat16, lo, hi)
    def permutation(self, n):
        return jax.random.permutation(self._next(), n)


kernel_name = 'concat_heads__sliding_local_dilated__sliding_block__prompt'

def setup_inputs():
    _rng = _Rng(jax.random.key(int.from_bytes(__import__("os").urandom(4), "little")))
    _w = (lambda a: (lambda t: t.astype(jnp.bfloat16) if jnp.issubdtype(t.dtype, jnp.floating) else t)(jnp.asarray(a)))
    def _A_setup():
        B, S, D = 1, 2048, 1024
        return {
            "x": _w((lambda *s: _rng.normal(s) * 0.2)(B, S, D)),
            "wqkv": _w((lambda *s: _rng.normal(s) * 0.2)(D, 3 * D)),
            "wo": _w((lambda *s: _rng.normal(s) * 0.05)(D, D)),
        }
    _A_in = _A_setup()

    def _B_setup():
        B, S, D = 1, 2048, 1024
        return {
            "x": _w((lambda *s: _rng.normal(s) * 0.2)(B, S, D)),
            "wqkv": _w((lambda *s: _rng.normal(s) * 0.2)(D, 3 * D)),
            "wo": _w((lambda *s: _rng.normal(s) * 0.05)(D, D)),
        }
    _B_in = _B_setup()

    return {
        "A_x": _A_in["x"],
        "A_wqkv": _A_in["wqkv"],
        "A_wo": _A_in["wo"],
        "B_x": _B_in["x"],
        "B_wqkv": _B_in["wqkv"],
        "B_wo": _B_in["wo"],
    }

def reference(A_x, A_wqkv, A_wo, B_x, B_wqkv, B_wo):
    def _A_ref(x, wqkv, wo):
        B, S, D = x.shape
        H = 32; Dh = D // H
        W, dil = 8, 2
        qkv = (lambda x, *d: x.transpose(*d))((x @ wqkv).reshape(B, S, 3, H, Dh), 2, 0, 3, 1, 4)
        q, k, v = qkv[0], qkv[1], qkv[2]
        scale = Dh ** -0.5
        pos = jnp.arange(S)
        off = jnp.arange(W) * dil
        idx = pos[:, None] - off[None, :]
        mask = idx >= 0
        idx_c = jnp.where(mask, idx, 0).reshape(-1)
        kg = k[:, :, idx_c, :].reshape(B, H, S, W, Dh)
        vg = v[:, :, idx_c, :].reshape(B, H, S, W, Dh)
        logits = jnp.einsum("bhsd,bhswd->bhsw", q, kg) * scale
        logits = jnp.where(mask[None, None, :, :], logits, -1e9)
        attn = _softmax(logits, axis=-1)
        o = jnp.einsum("bhsw,bhswd->bhsd", attn, vg)
        return (lambda x, *d: x.transpose(*d))(o, 0, 2, 1, 3).reshape(B, S, D) @ wo

    def _B_ref(x, wqkv, wo):
        B, S, D = x.shape
        H = 32; Dh = D // H; W = 256
        qkv = (lambda x, *d: x.transpose(*d))((x @ wqkv).reshape(B, S, 3, H, Dh), 2, 0, 3, 1, 4)
        q, k, v = qkv[0], qkv[1], qkv[2]
        scores = jnp.einsum("bhqd,bhkd->bhqk", q, k) * (Dh ** -0.5)
        idx = jnp.arange(S)
        mask = (idx[:, None] - idx[None, :] >= 0) & (idx[:, None] - idx[None, :] < W)
        scores = jnp.where(mask[None, None], scores, -1e9)
        p = _softmax(scores, axis=-1)
        o = jnp.einsum("bhqk,bhkd->bhqd", p, v)
        return (lambda x, *d: x.transpose(*d))(o, 0, 2, 1, 3).reshape(B, S, D) @ wo

    a = _A_ref(A_x, A_wqkv, A_wo)
    b = _B_ref(B_x, B_wqkv, B_wo)
    return jnp.concatenate([a, b], axis=-1)
```

```python
import jax
import jax.numpy as jnp
from jax import lax
import jax.experimental.pallas as pl
import jax.experimental.pallas.tpu as pltpu

S = 2048
D = 1024
H = 32
DH = 32
T = 256
NSTEP = S // T
WIN_B = 256
W_A = 8
DIL = 2
HIST_A = 16
NEG = -1e9
SCALE = DH ** -0.5
RC = 64
RA = 16


def _permute_qkv_cols(w_ref, wp_ref):
    lane = lax.broadcasted_iota(jnp.int32, (RC // 2, 128), 1)

    def body(i, carry):
        r0 = pl.multiple_of(i * RC, RC)
        for part in range(3):
            tiles = [
                pltpu.bitcast(
                    w_ref[pl.ds(r0, RC), pl.ds(part * D + t * 128, 128)], jnp.uint32)
                for t in range(8)
            ]
            for k in range(3):
                p = k + 2
                sh = 1 << p
                low = ((lane >> p) & 1) == 0
                new = list(tiles)
                for t in range(8):
                    if t & (1 << k):
                        continue
                    a = tiles[t]
                    b = tiles[t | (1 << k)]
                    new[t] = jnp.where(low, a, pltpu.roll(b, sh, 1))
                    new[t | (1 << k)] = jnp.where(low, pltpu.roll(a, 128 - sh, 1), b)
                tiles = new
            for (p, q) in ((6, 1), (5, 0)):
                dist = (1 << p) - (1 << q)
                bp = (lane >> p) & 1
                bq = (lane >> q) & 1
                same = bp == bq
                hi = bp == 1
                tiles = [
                    jnp.where(same, x,
                              jnp.where(hi, pltpu.roll(x, dist, 1),
                                        pltpu.roll(x, 128 - dist, 1)))
                    for x in tiles
                ]
            for t in range(8):
                wp_ref[pl.ds(r0, RC), pl.ds(part * D + t * 128, 128)] = (
                    pltpu.bitcast(tiles[t], jnp.bfloat16))
        return carry

    lax.fori_loop(0, D // RC, body, 0)


def _kernel(xa_ref, wqa_ref, woa_ref, xb_ref, wqb_ref, wob_ref, out_ref,
            wqa_p, woa_p, wo32, qa_scr, ka_buf, va_buf, oa_scr,
            qb_scr, kb_all, vb_all, ob_scr):
    step = pl.program_id(0)

    @pl.when(step == 0)
    def _init():
        _permute_qkv_cols(wqa_ref, wqa_p)
        for j in range(8):
            wo32[j] = woa_ref[:, j * 128:(j + 1) * 128].astype(jnp.float32)
        for j in range(8):
            for d in range(DH):
                woa_p[d * H:(d + 1) * H, j * 128:(j + 1) * 128] = (
                    wo32[j, pl.ds(d, H, stride=DH), :].astype(jnp.bfloat16))
        ka_buf[0:HIST_A, :] = jnp.zeros((HIST_A, D), jnp.float32)
        va_buf[0:HIST_A, :] = jnp.zeros((HIST_A, D), jnp.float32)
        kb_all[:, 0:WIN_B, :] = jnp.zeros((8, WIN_B, 128), jnp.bfloat16)
        vb_all[:, 0:WIN_B, :] = jnp.zeros((8, WIN_B, 128), jnp.bfloat16)

    qkv = jnp.dot(xa_ref[...], wqa_p[...], preferred_element_type=jnp.float32)
    qa_scr[...] = qkv[:, 0:D] * SCALE
    ka_buf[HIST_A:HIST_A + T, :] = qkv[:, D:2 * D]
    va_buf[HIST_A:HIST_A + T, :] = qkv[:, 2 * D:3 * D]

    qkv = jnp.dot(xb_ref[...], wqb_ref[...], preferred_element_type=jnp.float32)
    krow = pl.multiple_of(step * T + WIN_B, 128)
    for g in range(8):
        qb_scr[g] = (qkv[:, g * 128:(g + 1) * 128] * SCALE).astype(jnp.bfloat16)
        kb_all[g, pl.ds(krow, T), :] = (
            qkv[:, D + g * 128:D + (g + 1) * 128].astype(jnp.bfloat16))
        vb_all[g, pl.ds(krow, T), :] = (
            qkv[:, 2 * D + g * 128:2 * D + (g + 1) * 128].astype(jnp.bfloat16))

    row_a = lax.broadcasted_iota(jnp.int32, (RA, 128), 0)

    def body_a(c, carry):
        r0 = pl.multiple_of(c * RA, RA)
        q = qa_scr[pl.ds(r0, RA), :]
        kk = ka_buf[pl.ds(r0, RA + HIST_A), :]
        vv = va_buf[pl.ds(r0, RA + HIST_A), :]
        pos = step * T + r0 + row_a
        logits = []
        for w in range(W_A):
            o = HIST_A - DIL * w
            prod = q * kk[o:o + RA, :]
            acc = prod[:, 0:128]
            for j in range(1, 8):
                acc = acc + prod[:, j * 128:(j + 1) * 128]
            acc = acc + pltpu.roll(acc, 64, 1)
            acc = acc + pltpu.roll(acc, 32, 1)
            if w > 0:
                acc = jnp.where(pos >= DIL * w, acc, NEG)
            logits.append(acc)
        m = logits[0]
        for w in range(1, W_A):
            m = jnp.maximum(m, logits[w])
        es = [jnp.exp(l - m) for l in logits]
        den = es[0]
        for w in range(1, W_A):
            den = den + es[w]
        inv = 1.0 / den
        out = None
        for w in range(W_A):
            o = HIST_A - DIL * w
            pw = es[w] * inv
            pw = jnp.concatenate([pw] * 8, axis=1)
            term = pw * vv[o:o + RA, :]
            out = term if out is None else out + term
        oa_scr[pl.ds(r0, RA), :] = out.astype(jnp.bfloat16)
        return carry

    lax.fori_loop(0, T // RA, body_a, 0)
    ka_buf[0:HIST_A, :] = ka_buf[T:T + HIST_A, :]
    va_buf[0:HIST_A, :] = va_buf[T:T + HIST_A, :]

    out_ref[:, 0:D] = jnp.dot(
        oa_scr[...], woa_p[...], preferred_element_type=jnp.float32
    ).astype(out_ref.dtype)

    lanehead = lax.broadcasted_iota(jnp.int32, (128, 128), 1) // DH
    r_i = lax.broadcasted_iota(jnp.int32, (512, 384), 0) % 128
    c_i = lax.broadcasted_iota(jnp.int32, (512, 384), 1) - WIN_B
    diff = r_i - c_i
    band = (diff >= 0) & (diff < WIN_B)

    for sb in range(T // 128):
        qrow = step * T + sb * 128
        valid = band & (c_i + qrow >= 0)
        kstart = pl.multiple_of(qrow, 128)

        def body_b(g, carry):
            q4 = qb_scr[g, sb * 128:(sb + 1) * 128, :]
            zero = jnp.zeros_like(q4)
            lhs = jnp.concatenate(
                [jnp.where(lanehead == h, q4, zero) for h in range(4)], axis=0)
            k3 = kb_all[g, pl.ds(kstart, 384), :]
            v3 = vb_all[g, pl.ds(kstart, 384), :]
            s = lax.dot_general(lhs, k3, (((1,), (1,)), ((), ())),
                                preferred_element_type=jnp.float32)
            s = jnp.where(valid, s, NEG)
            m = jnp.max(s, axis=1, keepdims=True)
            p = jnp.exp(s - m)
            l = jnp.sum(p, axis=1, keepdims=True)
            r = jnp.dot(p.astype(jnp.bfloat16), v3,
                        preferred_element_type=jnp.float32)
            r = r * (1.0 / l)
            o4 = jnp.where(lanehead == 0, r[0:128], 0.0)
            for h in range(1, 4):
                o4 = jnp.where(lanehead == h, r[h * 128:(h + 1) * 128], o4)
            ob_scr[g, sb * 128:(sb + 1) * 128, :] = o4.astype(jnp.bfloat16)
            return carry

        lax.fori_loop(0, 8, body_b, 0)

    ob = jnp.concatenate([ob_scr[g] for g in range(8)], axis=1)
    out_ref[:, D:2 * D] = jnp.dot(
        ob, wob_ref[...], preferred_element_type=jnp.float32
    ).astype(out_ref.dtype)


@jax.jit
def pallas_concat_heads__sliding_local_dilated__sliding_block__prompt_kernel(
    A_x: jax.Array,
    A_wqkv: jax.Array,
    A_wo: jax.Array,
    B_x: jax.Array,
    B_wqkv: jax.Array,
    B_wo: jax.Array,
):
    xa = A_x.reshape(S, D)
    xb = B_x.reshape(S, D)
    const = lambda i: (0, 0)
    out = pl.pallas_call(
        _kernel,
        grid=(NSTEP,),
        in_specs=[
            pl.BlockSpec((T, D), lambda i: (i, 0)),
            pl.BlockSpec((D, 3 * D), const),
            pl.BlockSpec((D, D), const),
            pl.BlockSpec((T, D), lambda i: (i, 0)),
            pl.BlockSpec((D, 3 * D), const),
            pl.BlockSpec((D, D), const),
        ],
        out_specs=pl.BlockSpec((T, 2 * D), lambda i: (i, 0)),
        out_shape=jax.ShapeDtypeStruct((S, 2 * D), jnp.bfloat16),
        scratch_shapes=[
            pltpu.VMEM((D, 3 * D), jnp.bfloat16),
            pltpu.VMEM((D, D), jnp.bfloat16),
            pltpu.VMEM((8, D, 128), jnp.float32),
            pltpu.VMEM((T, D), jnp.float32),
            pltpu.VMEM((T + HIST_A, D), jnp.float32),
            pltpu.VMEM((T + HIST_A, D), jnp.float32),
            pltpu.VMEM((T, D), jnp.bfloat16),
            pltpu.VMEM((8, T, 128), jnp.bfloat16),
            pltpu.VMEM((8, S + WIN_B, 128), jnp.bfloat16),
            pltpu.VMEM((8, S + WIN_B, 128), jnp.bfloat16),
            pltpu.VMEM((8, T, 128), jnp.bfloat16),
        ],
        compiler_params=pltpu.CompilerParams(
            dimension_semantics=("arbitrary",),
            vmem_limit_bytes=100 * 1024 * 1024,
        ),
    )(xa, A_wqkv, A_wo, xb, B_wqkv, B_wo)
    return out.reshape(1, S, 2 * D)
```

```python
import jax
import jax.numpy as jnp
from jax import lax
import jax.experimental.pallas as pl
import jax.experimental.pallas.tpu as pltpu

S = 2048
D = 1024
H = 32
DH = 32
T = 256
NSTEP = S // T
WIN_B = 256
W_A = 8
DIL = 2
HIST_A = 16
NEG = -1e9
SCALE = DH ** -0.5
RC = 128
START_B = 5
RA = 8


def _permute_qkv_rows(w_ref, r0):
    lane = lax.broadcasted_iota(jnp.int32, (RC // 2, 128), 1)
    tiles = {}

    def load(part):
        tiles[part] = [
            pltpu.bitcast(
                w_ref[pl.ds(r0, RC), pl.ds(part * D + t * 128, 128)], jnp.uint32)
            for t in range(8)
        ]

    def stage(part, k):
        p = k + 2
        sh = 1 << p
        low = ((lane >> p) & 1) == 0
        cur = tiles[part]
        new = list(cur)
        for t in range(8):
            if t & (1 << k):
                continue
            a = cur[t]
            b = cur[t | (1 << k)]
            new[t] = jnp.where(low, a, pltpu.roll(b, sh, 1))
            new[t | (1 << k)] = jnp.where(low, pltpu.roll(a, 128 - sh, 1), b)
        tiles[part] = new

    def store(part):
        for t in range(8):
            w_ref[pl.ds(r0, RC), pl.ds(part * D + t * 128, 128)] = (
                pltpu.bitcast(tiles[part][t], jnp.bfloat16))

    for slot in range(5):
        for part in range(3):
            k = slot - part
            if k == 0:
                load(part)
            if 0 <= k < 3:
                stage(part, k)
            if k == 2:
                store(part)


def _attn_a_rows(step, r0, qa_scr, ka_buf, va_buf, oa_scr):
    row_a = lax.broadcasted_iota(jnp.int32, (RA, 128), 0)
    pos = step * T + r0 + row_a
    lane_a = lax.broadcasted_iota(jnp.int32, (RA, 128), 1)
    odd1 = (lane_a & 1) == 1
    odd2 = (lane_a & 2) == 2
    q = [qa_scr[j, r0:r0 + RA, :] for j in range(8)]
    logits = []
    for w in range(W_A):
        o = r0 + HIST_A - DIL * w
        acc = q[0] * ka_buf[0, o:o + RA, :]
        for j in range(1, 8):
            acc = acc + q[j] * ka_buf[j, o:o + RA, :]
        logits.append(acc)
    logits = [a + jnp.where(odd1, pltpu.roll(a, 1, 1), pltpu.roll(a, 127, 1))
              for a in logits]
    logits = [a + jnp.where(odd2, pltpu.roll(a, 2, 1), pltpu.roll(a, 126, 1))
              for a in logits]
    for w in range(1, W_A):
        if r0 < DIL * w:
            logits[w] = jnp.where(pos >= DIL * w, logits[w], NEG)
    m = logits[0]
    for w in range(1, W_A):
        m = jnp.maximum(m, logits[w])
    es = [jnp.exp(l - m) for l in logits]
    den = es[0]
    for w in range(1, W_A):
        den = den + es[w]
    inv = 1.0 / den
    ps = [e * inv for e in es]
    for j in range(8):
        out = None
        for w in range(W_A):
            o = r0 + HIST_A - DIL * w
            term = ps[w] * va_buf[j, o:o + RA, :]
            out = term if out is None else out + term
        oa_scr[r0:r0 + RA, j * 128:(j + 1) * 128] = out.astype(jnp.bfloat16)


def _b_scores(step, g, qb_scr, kb_all):
    lanehead = lax.broadcasted_iota(jnp.int32, (128, 128), 1) // DH
    out = []
    for sb in range(T // 128):
        kstart = pl.multiple_of((step * (T // 128) + sb) * 128, 128)
        q4 = qb_scr[g, sb * 128:(sb + 1) * 128, :]
        zero = jnp.zeros_like(q4)
        k3 = kb_all[g, pl.ds(kstart, 384), :]
        for h in range(4):
            qm = jnp.where(lanehead == h, q4, zero)
            out.append(lax.dot_general(k3, qm, (((1,), (1,)), ((), ())),
                                       preferred_element_type=jnp.float32))
    return out


def _b_softmax_pv(step, g, scores, vbt_all, ob_scr):
    key_i = lax.broadcasted_iota(jnp.int32, (128, 128), 0)
    qry_i = lax.broadcasted_iota(jnp.int32, (128, 128), 1)
    tri = key_i <= qry_i
    ps, ls = [], []
    for sb in range(T // 128):
        gsb = step * (T // 128) + sb
        b0 = jnp.where(gsb < 2, NEG, 0.0).astype(jnp.float32)
        b1 = jnp.where(gsb < 1, NEG, 0.0).astype(jnp.float32)
        for h in range(4):
            s = scores[sb * 4 + h]
            sc = jnp.where(tri, s[256:384], s[0:128] + b0)
            s1 = s[128:256]
            if sb == 0:
                s1 = s1 + b1
            m = jnp.max(jnp.maximum(sc, s1), axis=0, keepdims=True)
            pc = jnp.exp(sc - m)
            p1 = jnp.exp(s1 - m)
            ls.append(jnp.sum(pc + p1, axis=0, keepdims=True))
            p = jnp.concatenate(
                [jnp.where(tri, 0.0, pc), p1, jnp.where(tri, pc, 0.0)], axis=0)
            ps.append(p.astype(jnp.bfloat16))
    for sb in range(T // 128):
        kstart = pl.multiple_of((step * (T // 128) + sb) * 128, 128)
        ots = []
        for h in range(4):
            vt = vbt_all[g, h * DH:(h + 1) * DH, pl.ds(kstart, 384)]
            ot = jnp.dot(vt, ps[sb * 4 + h], preferred_element_type=jnp.float32)
            ots.append(ot * (1.0 / ls[sb * 4 + h]))
        o4 = jnp.concatenate(ots, axis=0).T
        ob_scr[sb * 128:(sb + 1) * 128, g * 128:(g + 1) * 128] = o4.astype(jnp.bfloat16)


def _kernel(xa_ref, wqa_hbm, woa_hbm, xb_ref, wqb_hbm, wob_hbm, out_ref,
            wqa_p, woa_raw, woa_p, wqb_ref, wob_ref, wo32,
            qa_scr, ka_buf, va_buf, oa_scr,
            qb_scr, kb_all, vb_all, ob_scr, sem_a, sem_w):
    step = pl.program_id(0)

    def wqa_copy(i):
        return pltpu.make_async_copy(
            wqa_hbm.at[pl.ds(i * RC, RC), :], wqa_p.at[pl.ds(i * RC, RC), :],
            sem_a.at[i])

    def w_copy(i):
        src, dst = ((wqb_hbm, wqb_ref), (woa_hbm, woa_raw), (wob_hbm, wob_ref))[i]
        return pltpu.make_async_copy(src, dst, sem_w.at[i])

    @pl.when(step == 0)
    def _init():
        for i in range(D // RC):
            wqa_copy(i).start()
        ka_buf[:, 0:HIST_A, :] = jnp.zeros((8, HIST_A, 128), jnp.float32)
        va_buf[:, 0:HIST_A, :] = jnp.zeros((8, HIST_A, 128), jnp.float32)
        kb_all[:, 0:WIN_B, :] = jnp.zeros((8, WIN_B, 128), jnp.bfloat16)
        vb_all[:, :, 0:WIN_B] = jnp.zeros((8, 128, WIN_B), jnp.bfloat16)

        def body(i, carry):
            wqa_copy(i).wait()

            @pl.when(i == START_B)
            def _():
                w_copy(0).start()

            _permute_qkv_rows(wqa_p, pl.multiple_of(i * RC, RC))
            return carry

        lax.fori_loop(0, D // RC, body, 0)
        w_copy(1).start()
        w_copy(2).start()

    xa = xa_ref[...]
    for j in range(8):
        qa_scr[j] = jnp.dot(xa, wqa_p[:, j * 128:(j + 1) * 128],
                            preferred_element_type=jnp.float32) * SCALE
        ka_buf[j, HIST_A:HIST_A + T, :] = jnp.dot(
            xa, wqa_p[:, D + j * 128:D + (j + 1) * 128],
            preferred_element_type=jnp.float32)
        va_buf[j, HIST_A:HIST_A + T, :] = jnp.dot(
            xa, wqa_p[:, 2 * D + j * 128:2 * D + (j + 1) * 128],
            preferred_element_type=jnp.float32)

    @pl.when(step == 0)
    def _wait_wqb():
        w_copy(0).wait()

    xb = xb_ref[...]
    krow = pl.multiple_of(step * T + WIN_B, 128)
    rows_per = T // 8
    for g in range(8):
        qb_scr[g] = (jnp.dot(xb, wqb_ref[:, g * 128:(g + 1) * 128],
                             preferred_element_type=jnp.float32) * SCALE
                     ).astype(jnp.bfloat16)
        kb_all[g, pl.ds(krow, T), :] = jnp.dot(
            xb, wqb_ref[:, D + g * 128:D + (g + 1) * 128],
            preferred_element_type=jnp.float32).astype(jnp.bfloat16)
        vb_all[g, :, pl.ds(krow, T)] = jnp.dot(
            xb, wqb_ref[:, 2 * D + g * 128:2 * D + (g + 1) * 128],
            preferred_element_type=jnp.float32).T.astype(jnp.bfloat16)
        for c in range(rows_per // RA):
            _attn_a_rows(step, g * rows_per + c * RA, qa_scr, ka_buf, va_buf, oa_scr)
    ka_buf[:, 0:HIST_A, :] = ka_buf[:, T:T + HIST_A, :]
    va_buf[:, 0:HIST_A, :] = va_buf[:, T:T + HIST_A, :]

    @pl.when(step == 0)
    def _prep_wo():
        w_copy(1).wait()
        for j in range(8):
            wo32[j] = woa_raw[:, j * 128:(j + 1) * 128].astype(jnp.float32)
        for j in range(8):
            for tile in range(8):
                for h0 in range(4):
                    rows = jnp.concatenate(
                        [wo32[j, pl.ds((h1 * 4 + h0) * DH + tile * 4, 4), :]
                         for h1 in range(8)], axis=0)
                    r0 = tile * 128 + h0 * 32
                    woa_p[r0:r0 + 32, j * 128:(j + 1) * 128] = rows.astype(jnp.bfloat16)
        w_copy(2).wait()

    oa = oa_scr[...]
    scores = _b_scores(step, 0, qb_scr, kb_all)
    for g in range(8):
        nxt = _b_scores(step, g + 1, qb_scr, kb_all) if g < 7 else None
        out_ref[:, g * 128:(g + 1) * 128] = jnp.dot(
            oa, woa_p[:, g * 128:(g + 1) * 128],
            preferred_element_type=jnp.float32).astype(out_ref.dtype)
        _b_softmax_pv(step, g, scores, vb_all, ob_scr)
        scores = nxt

    out_ref[:, D:2 * D] = jnp.dot(
        ob_scr[...], wob_ref[...], preferred_element_type=jnp.float32
    ).astype(out_ref.dtype)


@jax.jit
def pallas_concat_heads__sliding_local_dilated__sliding_block__prompt_kernel(
    A_x: jax.Array,
    A_wqkv: jax.Array,
    A_wo: jax.Array,
    B_x: jax.Array,
    B_wqkv: jax.Array,
    B_wo: jax.Array,
):
    xa = A_x.reshape(S, D)
    xb = B_x.reshape(S, D)
    out = pl.pallas_call(
        _kernel,
        grid=(NSTEP,),
        in_specs=[
            pl.BlockSpec((T, D), lambda i: (i, 0)),
            pl.BlockSpec(memory_space=pl.ANY),
            pl.BlockSpec(memory_space=pl.ANY),
            pl.BlockSpec((T, D), lambda i: (i, 0)),
            pl.BlockSpec(memory_space=pl.ANY),
            pl.BlockSpec(memory_space=pl.ANY),
        ],
        out_specs=pl.BlockSpec((T, 2 * D), lambda i: (i, 0)),
        out_shape=jax.ShapeDtypeStruct((S, 2 * D), jnp.bfloat16),
        scratch_shapes=[
            pltpu.VMEM((D, 3 * D), jnp.bfloat16),
            pltpu.VMEM((D, D), jnp.bfloat16),
            pltpu.VMEM((D, D), jnp.bfloat16),
            pltpu.VMEM((D, 3 * D), jnp.bfloat16),
            pltpu.VMEM((D, D), jnp.bfloat16),
            pltpu.VMEM((8, D, 128), jnp.float32),
            pltpu.VMEM((8, T, 128), jnp.float32),
            pltpu.VMEM((8, T + HIST_A, 128), jnp.float32),
            pltpu.VMEM((8, T + HIST_A, 128), jnp.float32),
            pltpu.VMEM((T, D), jnp.bfloat16),
            pltpu.VMEM((8, T, 128), jnp.bfloat16),
            pltpu.VMEM((8, S + WIN_B, 128), jnp.bfloat16),
            pltpu.VMEM((8, 128, S + WIN_B), jnp.bfloat16),
            pltpu.VMEM((T, D), jnp.bfloat16),
            pltpu.SemaphoreType.DMA((D // RC,)),
            pltpu.SemaphoreType.DMA((3,)),
        ],
        compiler_params=pltpu.CompilerParams(
            dimension_semantics=("arbitrary",),
            vmem_limit_bytes=100 * 1024 * 1024,
        ),
    )(xa, A_wqkv, A_wo, xb, B_wqkv, B_wo)
    return out.reshape(1, S, 2 * D)
```

```python
import jax
import jax.numpy as jnp
from jax import lax
import jax.experimental.pallas as pl
import jax.experimental.pallas.tpu as pltpu

S = 2048
D = 1024
H = 32
DH = 32
T = 256
NSTEP = S // T
WIN_B = 256
W_A = 8
DIL = 2
HIST_A = 16
NEG = -1e9
SCALE = DH ** -0.5
SCALE_LOG2E = SCALE * 1.4426950408889634
RC = 128
START_B = 5
RA = 8


def _permute_qkv_rows(w_ref, r0):
    lane = lax.broadcasted_iota(jnp.int32, (RC // 2, 128), 1)
    tiles = {}

    def load(part):
        tiles[part] = [
            pltpu.bitcast(
                w_ref[pl.ds(r0, RC), pl.ds(part * D + t * 128, 128)], jnp.uint32)
            for t in range(8)
        ]

    def stage(part, k):
        p = k + 2
        sh = 1 << p
        low = ((lane >> p) & 1) == 0
        cur = tiles[part]
        new = list(cur)
        for t in range(8):
            if t & (1 << k):
                continue
            a = cur[t]
            b = cur[t | (1 << k)]
            new[t] = jnp.where(low, a, pltpu.roll(b, sh, 1))
            new[t | (1 << k)] = jnp.where(low, pltpu.roll(a, 128 - sh, 1), b)
        tiles[part] = new

    def store(part):
        for t in range(8):
            w_ref[pl.ds(r0, RC), pl.ds(part * D + t * 128, 128)] = (
                pltpu.bitcast(tiles[part][t], jnp.bfloat16))

    for slot in range(5):
        for part in range(3):
            k = slot - part
            if k == 0:
                load(part)
            if 0 <= k < 3:
                stage(part, k)
            if k == 2:
                store(part)


def _attn_a_rows(step, r0, qa_scr, ka_buf, va_buf, oa_scr):
    row_a = lax.broadcasted_iota(jnp.int32, (RA, 128), 0)
    pos = step * T + r0 + row_a
    lane_a = lax.broadcasted_iota(jnp.int32, (RA, 128), 1)
    odd1 = (lane_a & 1) == 1
    odd2 = (lane_a & 2) == 2
    q = [qa_scr[j, r0:r0 + RA, :] for j in range(8)]
    logits = []
    for w in range(W_A):
        o = r0 + HIST_A - DIL * w
        acc = q[0] * ka_buf[0, o:o + RA, :]
        for j in range(1, 8):
            acc = acc + q[j] * ka_buf[j, o:o + RA, :]
        logits.append(acc)
    logits = [a + jnp.where(odd1, pltpu.roll(a, 1, 1), pltpu.roll(a, 127, 1))
              for a in logits]
    logits = [a + jnp.where(odd2, pltpu.roll(a, 2, 1), pltpu.roll(a, 126, 1))
              for a in logits]
    for w in range(1, W_A):
        if r0 < DIL * w:
            logits[w] = jnp.where(pos >= DIL * w, logits[w], NEG)
    m = logits[0]
    for w in range(1, W_A):
        m = jnp.maximum(m, logits[w])
    es = [jnp.exp(l - m) for l in logits]
    den = es[0]
    for w in range(1, W_A):
        den = den + es[w]
    inv = 1.0 / den
    ps = [e * inv for e in es]
    for j in range(8):
        out = None
        for w in range(W_A):
            o = r0 + HIST_A - DIL * w
            term = ps[w] * va_buf[j, o:o + RA, :]
            out = term if out is None else out + term
        oa_scr[r0:r0 + RA, j * 128:(j + 1) * 128] = out.astype(jnp.bfloat16)


def _b_score_unit(step, g, sb, h, qb_scr, kb_all):
    lanehead = lax.broadcasted_iota(jnp.int32, (128, 128), 1) // DH
    kstart = pl.multiple_of((step * (T // 128) + sb) * 128, 128)
    q4 = qb_scr[g, sb * 128:(sb + 1) * 128, :]
    k3 = kb_all[g, pl.ds(kstart, 384), :]
    qm = jnp.where(lanehead == h, q4, jnp.zeros_like(q4))
    return lax.dot_general(k3, qm, (((1,), (1,)), ((), ())),
                           preferred_element_type=jnp.float32)


def _b_softmax_pv_unit(step, g, sb, h, s, vbt_all):
    key_i = lax.broadcasted_iota(jnp.int32, (128, 128), 0)
    qry_i = lax.broadcasted_iota(jnp.int32, (128, 128), 1)
    tri = key_i <= qry_i
    gsb = step * (T // 128) + sb
    b0 = jnp.where(gsb < 2, NEG, 0.0).astype(jnp.float32)
    b1 = jnp.where(gsb < 1, NEG, 0.0).astype(jnp.float32)
    sc = jnp.where(tri, s[256:384], s[0:128] + b0)
    s1 = s[128:256]
    if sb == 0:
        s1 = s1 + b1
    m = jnp.max(jnp.maximum(sc, s1), axis=0, keepdims=True)
    pc = jnp.exp2(sc - m)
    p1 = jnp.exp2(s1 - m)
    l = jnp.sum(pc + p1, axis=0, keepdims=True)
    p = jnp.concatenate(
        [jnp.where(tri, 0.0, pc), p1, jnp.where(tri, pc, 0.0)], axis=0)
    kstart = pl.multiple_of(gsb * 128, 128)
    vt = vbt_all[g, h * DH:(h + 1) * DH, pl.ds(kstart, 384)]
    ot = jnp.dot(vt, p.astype(jnp.bfloat16), preferred_element_type=jnp.float32)
    return ot * (1.0 / l)


def _kernel(xa_ref, wqa_hbm, woa_hbm, xb_ref, wqb_hbm, wob_hbm, out_ref,
            wqa_p, woa_raw, woa_p, wqb_ref, wob_ref, wo32,
            qa_scr, ka_buf, va_buf, oa_scr,
            qb_scr, kb_all, vb_all, ob_scr, sem_a, sem_w):
    step = pl.program_id(0)

    def wqa_copy(i):
        return pltpu.make_async_copy(
            wqa_hbm.at[pl.ds(i * RC, RC), :], wqa_p.at[pl.ds(i * RC, RC), :],
            sem_a.at[i])

    def w_copy(i):
        src, dst = ((wqb_hbm, wqb_ref), (woa_hbm, woa_raw), (wob_hbm, wob_ref))[i]
        return pltpu.make_async_copy(src, dst, sem_w.at[i])

    @pl.when(step == 0)
    def _init():
        for i in range(D // RC):
            wqa_copy(i).start()
        ka_buf[:, 0:HIST_A, :] = jnp.zeros((8, HIST_A, 128), jnp.float32)
        va_buf[:, 0:HIST_A, :] = jnp.zeros((8, HIST_A, 128), jnp.float32)
        kb_all[:, 0:WIN_B, :] = jnp.zeros((8, WIN_B, 128), jnp.bfloat16)
        vb_all[:, :, 0:WIN_B] = jnp.zeros((8, 128, WIN_B), jnp.bfloat16)

        def body(i, carry):
            wqa_copy(i).wait()

            @pl.when(i == START_B)
            def _():
                w_copy(0).start()

            _permute_qkv_rows(wqa_p, pl.multiple_of(i * RC, RC))
            return carry

        lax.fori_loop(0, D // RC, body, 0)
        w_copy(1).start()
        w_copy(2).start()

    xa = xa_ref[...]
    for j in range(8):
        qa_scr[j] = jnp.dot(xa, wqa_p[:, j * 128:(j + 1) * 128],
                            preferred_element_type=jnp.float32) * SCALE
        ka_buf[j, HIST_A:HIST_A + T, :] = jnp.dot(
            xa, wqa_p[:, D + j * 128:D + (j + 1) * 128],
            preferred_element_type=jnp.float32)
        va_buf[j, HIST_A:HIST_A + T, :] = jnp.dot(
            xa, wqa_p[:, 2 * D + j * 128:2 * D + (j + 1) * 128],
            preferred_element_type=jnp.float32)

    @pl.when(step == 0)
    def _wait_wqb():
        w_copy(0).wait()

    xb = xb_ref[...]
    krow = pl.multiple_of(step * T + WIN_B, 128)
    rows_per = T // 8
    for g in range(8):
        qb_scr[g] = (jnp.dot(xb, wqb_ref[:, g * 128:(g + 1) * 128],
                             preferred_element_type=jnp.float32) * SCALE_LOG2E
                     ).astype(jnp.bfloat16)
        _attn_a_rows(step, g * rows_per + 0 * RA, qa_scr, ka_buf, va_buf, oa_scr)
        kb_all[g, pl.ds(krow, T), :] = jnp.dot(
            xb, wqb_ref[:, D + g * 128:D + (g + 1) * 128],
            preferred_element_type=jnp.float32).astype(jnp.bfloat16)
        _attn_a_rows(step, g * rows_per + 1 * RA, qa_scr, ka_buf, va_buf, oa_scr)
        _attn_a_rows(step, g * rows_per + 2 * RA, qa_scr, ka_buf, va_buf, oa_scr)
        vb_all[g, :, pl.ds(krow, T)] = jnp.dot(
            xb, wqb_ref[:, 2 * D + g * 128:2 * D + (g + 1) * 128],
            preferred_element_type=jnp.float32).T.astype(jnp.bfloat16)
        _attn_a_rows(step, g * rows_per + 3 * RA, qa_scr, ka_buf, va_buf, oa_scr)
    ka_buf[:, 0:HIST_A, :] = ka_buf[:, T:T + HIST_A, :]
    va_buf[:, 0:HIST_A, :] = va_buf[:, T:T + HIST_A, :]

    @pl.when(step == 0)
    def _prep_wo():
        w_copy(1).wait()
        for j in range(8):
            wo32[j] = woa_raw[:, j * 128:(j + 1) * 128].astype(jnp.float32)
        for j in range(8):
            for tile in range(8):
                for h0 in range(4):
                    rows = jnp.concatenate(
                        [wo32[j, pl.ds((h1 * 4 + h0) * DH + tile * 4, 4), :]
                         for h1 in range(8)], axis=0)
                    r0 = tile * 128 + h0 * 32
                    woa_p[r0:r0 + 32, j * 128:(j + 1) * 128] = rows.astype(jnp.bfloat16)
        w_copy(2).wait()

    units = [(g, sb, h) for g in range(8) for sb in range(T // 128) for h in range(4)]
    LOOK = 8
    pend = [_b_score_unit(step, *units[i], qb_scr, kb_all) for i in range(LOOK)]
    acc = None
    ots = []
    for i, (g, sb, h) in enumerate(units):
        if i + LOOK < len(units):
            pend.append(_b_score_unit(step, *units[i + LOOK], qb_scr, kb_all))
        kt = sb * 4 + h
        part = jnp.dot(oa_scr[:, kt * 128:(kt + 1) * 128],
                       woa_p[kt * 128:(kt + 1) * 128, g * 128:(g + 1) * 128],
                       preferred_element_type=jnp.float32)
        acc = part if kt == 0 else acc + part
        if kt == 7:
            out_ref[:, g * 128:(g + 1) * 128] = acc.astype(out_ref.dtype)
        ots.append(_b_softmax_pv_unit(step, g, sb, h, pend.pop(0), vb_all))
        if h == 3:
            o4 = jnp.concatenate(ots, axis=0).T
            ob_scr[sb * 128:(sb + 1) * 128, g * 128:(g + 1) * 128] = (
                o4.astype(jnp.bfloat16))
            ots = []

    out_ref[:, D:2 * D] = jnp.dot(
        ob_scr[...], wob_ref[...], preferred_element_type=jnp.float32
    ).astype(out_ref.dtype)


@jax.jit
def pallas_concat_heads__sliding_local_dilated__sliding_block__prompt_kernel(
    A_x: jax.Array,
    A_wqkv: jax.Array,
    A_wo: jax.Array,
    B_x: jax.Array,
    B_wqkv: jax.Array,
    B_wo: jax.Array,
):
    xa = A_x.reshape(S, D)
    xb = B_x.reshape(S, D)
    out = pl.pallas_call(
        _kernel,
        grid=(NSTEP,),
        in_specs=[
            pl.BlockSpec((T, D), lambda i: (i, 0)),
            pl.BlockSpec(memory_space=pl.ANY),
            pl.BlockSpec(memory_space=pl.ANY),
            pl.BlockSpec((T, D), lambda i: (i, 0)),
            pl.BlockSpec(memory_space=pl.ANY),
            pl.BlockSpec(memory_space=pl.ANY),
        ],
        out_specs=pl.BlockSpec((T, 2 * D), lambda i: (i, 0)),
        out_shape=jax.ShapeDtypeStruct((S, 2 * D), jnp.bfloat16),
        scratch_shapes=[
            pltpu.VMEM((D, 3 * D), jnp.bfloat16),
            pltpu.VMEM((D, D), jnp.bfloat16),
            pltpu.VMEM((D, D), jnp.bfloat16),
            pltpu.VMEM((D, 3 * D), jnp.bfloat16),
            pltpu.VMEM((D, D), jnp.bfloat16),
            pltpu.VMEM((8, D, 128), jnp.float32),
            pltpu.VMEM((8, T, 128), jnp.float32),
            pltpu.VMEM((8, T + HIST_A, 128), jnp.float32),
            pltpu.VMEM((8, T + HIST_A, 128), jnp.float32),
            pltpu.VMEM((T, D), jnp.bfloat16),
            pltpu.VMEM((8, T, 128), jnp.bfloat16),
            pltpu.VMEM((8, S + WIN_B, 128), jnp.bfloat16),
            pltpu.VMEM((8, 128, S + WIN_B), jnp.bfloat16),
            pltpu.VMEM((T, D), jnp.bfloat16),
            pltpu.SemaphoreType.DMA((D // RC,)),
            pltpu.SemaphoreType.DMA((3,)),
        ],
        compiler_params=pltpu.CompilerParams(
            dimension_semantics=("arbitrary",),
            vmem_limit_bytes=100 * 1024 * 1024,
        ),
    )(xa, A_wqkv, A_wo, xb, B_wqkv, B_wo)
    return out.reshape(1, S, 2 * D)
```

```python
import jax
import jax.numpy as jnp
from jax import lax
import jax.experimental.pallas as pl
import jax.experimental.pallas.tpu as pltpu

S = 2048
D = 1024
H = 32
DH = 32
T = 256
NSTEP = S // T
WIN_B = 256
W_A = 8
DIL = 2
HIST_A = 16
NEG = -1e9
SCALE = DH ** -0.5
SCALE_LOG2E = SCALE * 1.4426950408889634
RC = 128
START_B = 3
RA = 8


def _permute_qkv_rows(w_ref, r0, use):
    lane = lax.broadcasted_iota(jnp.int32, (RC // 2, 128), 1)
    tiles = {}

    def load(part):
        tiles[part] = [
            pltpu.bitcast(
                w_ref[pl.ds(r0, RC), pl.ds(part * D + t * 128, 128)], jnp.uint32)
            for t in range(8)
        ]

    def stage(part, k):
        p = k + 2
        sh = 1 << p
        low = ((lane >> p) & 1) == 0
        cur = tiles[part]
        new = list(cur)
        for t in range(8):
            if t & (1 << k):
                continue
            a = cur[t]
            b = cur[t | (1 << k)]
            new[t] = jnp.where(low, a, pltpu.roll(b, sh, 1))
            new[t | (1 << k)] = jnp.where(low, pltpu.roll(a, 128 - sh, 1), b)
        tiles[part] = new

    def store(part):
        for t in range(8):
            wt = pltpu.bitcast(tiles[part][t], jnp.bfloat16)
            w_ref[pl.ds(r0, RC), pl.ds(part * D + t * 128, 128)] = wt
            use(part, t, wt)

    for slot in range(5):
        for part in range(3):
            k = slot - part
            if k == 0:
                load(part)
            if 0 <= k < 3:
                stage(part, k)
            if k == 2:
                store(part)


def _attn_a_rows(step, r0, qa_scr, ka_buf, va_buf, oa_scr):
    row_a = lax.broadcasted_iota(jnp.int32, (RA, 128), 0)
    pos = step * T + r0 + row_a
    lane_a = lax.broadcasted_iota(jnp.int32, (RA, 128), 1)
    odd1 = (lane_a & 1) == 1
    odd2 = (lane_a & 2) == 2
    q = [qa_scr[j, r0:r0 + RA, :] for j in range(8)]
    logits = []
    for w in range(W_A):
        o = r0 + HIST_A - DIL * w
        acc = q[0] * ka_buf[0, o:o + RA, :]
        for j in range(1, 8):
            acc = acc + q[j] * ka_buf[j, o:o + RA, :]
        logits.append(acc)
    logits = [a + jnp.where(odd1, pltpu.roll(a, 1, 1), pltpu.roll(a, 127, 1))
              for a in logits]
    logits = [a + jnp.where(odd2, pltpu.roll(a, 2, 1), pltpu.roll(a, 126, 1))
              for a in logits]
    for w in range(1, W_A):
        if r0 < DIL * w:
            logits[w] = jnp.where(pos >= DIL * w, logits[w], NEG)
    m = logits[0]
    for w in range(1, W_A):
        m = jnp.maximum(m, logits[w])
    es = [jnp.exp(l - m) for l in logits]
    den = es[0]
    for w in range(1, W_A):
        den = den + es[w]
    inv = 1.0 / den
    ps = [e * inv for e in es]
    for j in range(8):
        out = None
        for w in range(W_A):
            o = r0 + HIST_A - DIL * w
            term = ps[w] * va_buf[j, o:o + RA, :]
            out = term if out is None else out + term
        oa_scr[r0:r0 + RA, j * 128:(j + 1) * 128] = out.astype(jnp.bfloat16)


def _b_score_unit(step, g, sb, h, qb_scr, kb_all):
    lanehead = lax.broadcasted_iota(jnp.int32, (128, 128), 1) // DH
    kstart = pl.multiple_of((step * (T // 128) + sb) * 128, 128)
    q4 = qb_scr[g, sb * 128:(sb + 1) * 128, :]
    k3 = kb_all[g, pl.ds(kstart, 384), :]
    qm = jnp.where(lanehead == h, q4, jnp.zeros_like(q4))
    return lax.dot_general(k3, qm, (((1,), (1,)), ((), ())),
                           preferred_element_type=jnp.float32)


def _b_softmax_pv_unit(step, g, sb, h, s, vbt_all):
    key_i = lax.broadcasted_iota(jnp.int32, (128, 128), 0)
    qry_i = lax.broadcasted_iota(jnp.int32, (128, 128), 1)
    tri = key_i <= qry_i
    gsb = step * (T // 128) + sb
    b0 = jnp.where(gsb < 2, NEG, 0.0).astype(jnp.float32)
    b1 = jnp.where(gsb < 1, NEG, 0.0).astype(jnp.float32)
    sc = jnp.where(tri, s[256:384], s[0:128] + b0)
    s1 = s[128:256]
    if sb == 0:
        s1 = s1 + b1
    m = jnp.max(jnp.maximum(sc, s1), axis=0, keepdims=True)
    pc = jnp.exp2(sc - m)
    p1 = jnp.exp2(s1 - m)
    l = jnp.sum(pc + p1, axis=0, keepdims=True)
    p = jnp.concatenate(
        [jnp.where(tri, 0.0, pc), p1, jnp.where(tri, pc, 0.0)], axis=0)
    kstart = pl.multiple_of(gsb * 128, 128)
    vt = vbt_all[g, h * DH:(h + 1) * DH, pl.ds(kstart, 384)]
    ot = jnp.dot(vt, p.astype(jnp.bfloat16), preferred_element_type=jnp.float32)
    return ot * (1.0 / l)


def _kernel(xa_ref, wqa_hbm, woa_hbm, xb_ref, wqb_hbm, wob_hbm, out_ref,
            wqa_p, woa_raw, woa_p, wqb_ref, wob_ref, wo32,
            qa_scr, ka_buf, va_buf, oa_scr,
            qb_scr, kb_all, vb_all, ob_scr, sem_a, sem_w, sem_b):
    step = pl.program_id(0)

    def wqa_copy(i):
        return pltpu.make_async_copy(
            wqa_hbm.at[pl.ds(i * RC, RC), :], wqa_p.at[pl.ds(i * RC, RC), :],
            sem_a.at[i])

    def w_copy(i):
        src, dst = ((woa_hbm, woa_raw), (wob_hbm, wob_ref))[i - 1]
        return pltpu.make_async_copy(src, dst, sem_w.at[i - 1])

    def wqb_copy(hh):
        c0, n = ((0, D), (D, 2 * D))[hh]
        return pltpu.make_async_copy(
            wqb_hbm.at[:, pl.ds(c0, n)], wqb_ref.at[:, pl.ds(c0, n)],
            sem_b.at[hh])

    def proj_qb():
        xb = xb_ref[...]
        for g in range(8):
            qb_scr[g] = (jnp.dot(xb, wqb_ref[:, g * 128:(g + 1) * 128],
                                 preferred_element_type=jnp.float32) * SCALE_LOG2E
                         ).astype(jnp.bfloat16)

    @pl.when(step == 0)
    def _init():
        for i in range(D // RC):
            wqa_copy(i).start()
        qa_scr[...] = jnp.zeros((8, T, 128), jnp.float32)
        ka_buf[...] = jnp.zeros((8, T + HIST_A, 128), jnp.float32)
        va_buf[...] = jnp.zeros((8, T + HIST_A, 128), jnp.float32)
        kb_all[:, 0:WIN_B, :] = jnp.zeros((8, WIN_B, 128), jnp.bfloat16)
        vb_all[:, :, 0:WIN_B] = jnp.zeros((8, 128, WIN_B), jnp.bfloat16)

        def body(i, carry):
            wqa_copy(i).wait()

            @pl.when(i == START_B)
            def _():
                wqb_copy(0).start()
                wqb_copy(1).start()

            r0 = pl.multiple_of(i * RC, RC)
            xc = xa_ref[:, pl.ds(r0, RC)]

            def use(part, t, wt):
                r = jnp.dot(xc, wt, preferred_element_type=jnp.float32)
                if part == 0:
                    qa_scr[t] += r * SCALE
                elif part == 1:
                    ka_buf[t, HIST_A:HIST_A + T, :] += r
                else:
                    va_buf[t, HIST_A:HIST_A + T, :] += r

            _permute_qkv_rows(wqa_p, r0, use)
            return carry

        lax.fori_loop(0, D // RC, body, 0)
        w_copy(1).start()
        w_copy(2).start()
        wqb_copy(0).wait()
        proj_qb()

    @pl.when(step > 0)
    def _proj_a():
        xa = xa_ref[...]
        for j in range(8):
            qa_scr[j] = jnp.dot(xa, wqa_p[:, j * 128:(j + 1) * 128],
                                preferred_element_type=jnp.float32) * SCALE
            ka_buf[j, HIST_A:HIST_A + T, :] = jnp.dot(
                xa, wqa_p[:, D + j * 128:D + (j + 1) * 128],
                preferred_element_type=jnp.float32)
            va_buf[j, HIST_A:HIST_A + T, :] = jnp.dot(
                xa, wqa_p[:, 2 * D + j * 128:2 * D + (j + 1) * 128],
                preferred_element_type=jnp.float32)
        proj_qb()

    @pl.when(step == 0)
    def _wait_wqb():
        wqb_copy(1).wait()

    xb = xb_ref[...]
    krow = pl.multiple_of(step * T + WIN_B, 128)
    rows_per = T // 8
    for g in range(8):
        kb_all[g, pl.ds(krow, T), :] = jnp.dot(
            xb, wqb_ref[:, D + g * 128:D + (g + 1) * 128],
            preferred_element_type=jnp.float32).astype(jnp.bfloat16)
        _attn_a_rows(step, g * rows_per + 0 * RA, qa_scr, ka_buf, va_buf, oa_scr)
        _attn_a_rows(step, g * rows_per + 1 * RA, qa_scr, ka_buf, va_buf, oa_scr)
        vb_all[g, :, pl.ds(krow, T)] = jnp.dot(
            xb, wqb_ref[:, 2 * D + g * 128:2 * D + (g + 1) * 128],
            preferred_element_type=jnp.float32).T.astype(jnp.bfloat16)
        _attn_a_rows(step, g * rows_per + 2 * RA, qa_scr, ka_buf, va_buf, oa_scr)
        _attn_a_rows(step, g * rows_per + 3 * RA, qa_scr, ka_buf, va_buf, oa_scr)
    ka_buf[:, 0:HIST_A, :] = ka_buf[:, T:T + HIST_A, :]
    va_buf[:, 0:HIST_A, :] = va_buf[:, T:T + HIST_A, :]

    @pl.when(step == 0)
    def _prep_wo():
        w_copy(1).wait()
        for j in range(8):
            wo32[j] = woa_raw[:, j * 128:(j + 1) * 128].astype(jnp.float32)
        for j in range(8):
            for tile in range(8):
                for h0 in range(4):
                    rows = jnp.concatenate(
                        [wo32[j, pl.ds((h1 * 4 + h0) * DH + tile * 4, 4), :]
                         for h1 in range(8)], axis=0)
                    r0 = tile * 128 + h0 * 32
                    woa_p[r0:r0 + 32, j * 128:(j + 1) * 128] = rows.astype(jnp.bfloat16)
        w_copy(2).wait()

    units = [(g, sb, h) for g in range(8) for sb in range(T // 128) for h in range(4)]
    LOOK = 8
    pend = [_b_score_unit(step, *units[i], qb_scr, kb_all) for i in range(LOOK)]
    acc = None
    ots = []
    for i, (g, sb, h) in enumerate(units):
        if i + LOOK < len(units):
            pend.append(_b_score_unit(step, *units[i + LOOK], qb_scr, kb_all))
        kt = sb * 4 + h
        part = jnp.dot(oa_scr[:, kt * 128:(kt + 1) * 128],
                       woa_p[kt * 128:(kt + 1) * 128, g * 128:(g + 1) * 128],
                       preferred_element_type=jnp.float32)
        acc = part if kt == 0 else acc + part
        if kt == 7:
            out_ref[:, g * 128:(g + 1) * 128] = acc.astype(out_ref.dtype)
        ots.append(_b_softmax_pv_unit(step, g, sb, h, pend.pop(0), vb_all))
        if h == 3:
            o4 = jnp.concatenate(ots, axis=0).T
            ob_scr[sb * 128:(sb + 1) * 128, g * 128:(g + 1) * 128] = (
                o4.astype(jnp.bfloat16))
            ots = []

    out_ref[:, D:2 * D] = jnp.dot(
        ob_scr[...], wob_ref[...], preferred_element_type=jnp.float32
    ).astype(out_ref.dtype)


@jax.jit
def pallas_concat_heads__sliding_local_dilated__sliding_block__prompt_kernel(
    A_x: jax.Array,
    A_wqkv: jax.Array,
    A_wo: jax.Array,
    B_x: jax.Array,
    B_wqkv: jax.Array,
    B_wo: jax.Array,
):
    xa = A_x.reshape(S, D)
    xb = B_x.reshape(S, D)
    out = pl.pallas_call(
        _kernel,
        grid=(NSTEP,),
        in_specs=[
            pl.BlockSpec((T, D), lambda i: (i, 0)),
            pl.BlockSpec(memory_space=pl.ANY),
            pl.BlockSpec(memory_space=pl.ANY),
            pl.BlockSpec((T, D), lambda i: (i, 0)),
            pl.BlockSpec(memory_space=pl.ANY),
            pl.BlockSpec(memory_space=pl.ANY),
        ],
        out_specs=pl.BlockSpec((T, 2 * D), lambda i: (i, 0)),
        out_shape=jax.ShapeDtypeStruct((S, 2 * D), jnp.bfloat16),
        scratch_shapes=[
            pltpu.VMEM((D, 3 * D), jnp.bfloat16),
            pltpu.VMEM((D, D), jnp.bfloat16),
            pltpu.VMEM((D, D), jnp.bfloat16),
            pltpu.VMEM((D, 3 * D), jnp.bfloat16),
            pltpu.VMEM((D, D), jnp.bfloat16),
            pltpu.VMEM((8, D, 128), jnp.float32),
            pltpu.VMEM((8, T, 128), jnp.float32),
            pltpu.VMEM((8, T + HIST_A, 128), jnp.float32),
            pltpu.VMEM((8, T + HIST_A, 128), jnp.float32),
            pltpu.VMEM((T, D), jnp.bfloat16),
            pltpu.VMEM((8, T, 128), jnp.bfloat16),
            pltpu.VMEM((8, S + WIN_B, 128), jnp.bfloat16),
            pltpu.VMEM((8, 128, S + WIN_B), jnp.bfloat16),
            pltpu.VMEM((T, D), jnp.bfloat16),
            pltpu.SemaphoreType.DMA((D // RC,)),
            pltpu.SemaphoreType.DMA((2,)),
            pltpu.SemaphoreType.DMA((2,)),
        ],
        compiler_params=pltpu.CompilerParams(
            dimension_semantics=("arbitrary",),
            vmem_limit_bytes=100 * 1024 * 1024,
        ),
    )(xa, A_wqkv, A_wo, xb, B_wqkv, B_wo)
    return out.reshape(1, S, 2 * D)
```
